```python
import os as _os
_os.environ.setdefault("JAX_PLATFORMS", "cpu")
import jax
import jax.numpy as jnp

def _softmax(x, axis=-1):
    return jax.nn.softmax(x, axis=axis)
def _gelu(x):
    return jax.nn.gelu(x, approximate=True)
def _silu(x):
    return jax.nn.silu(x)
def _sigmoid(x):
    return jax.nn.sigmoid(x)
def _layernorm(x, axis=-1, eps=1e-5):
    m = jnp.mean(x, axis=axis, keepdims=True)
    v = jnp.var(x, axis=axis, keepdims=True)
    return (x - m) / jnp.sqrt(v + eps)
def _scatter_add(tgt, idx, src, axis=0):
    return tgt.at[idx].add(src)
def _segment_sum(src, seg, n):
    return jax.ops.segment_sum(src, seg, n)
class _Rng:
    def __init__(self, key):
        self._k = key
    def _next(self):
        self._k, sub = jax.random.split(self._k)
        return sub
    def normal(self, shape):
        return jax.random.normal(self._next(), shape, dtype=jnp.bfloat16)
    def randint(self, lo, hi, shape):
        return jax.random.randint(self._next(), shape, lo, hi, dtype=jnp.int32)
    def uniform(self, shape, lo=0.0, hi=1.0):
        return jax.random.uniform(self._next(), shape, jnp.bfloat16, lo, hi)
    def permutation(self, n):
        return jax.random.permutation(self._next(), n)


kernel_name = 'standalone__gqa_softmax__near_ridge'

def setup_inputs():
    _rng = _Rng(jax.random.key(int.from_bytes(__import__("os").urandom(4), "little")))
    _w = (lambda a: (lambda t: t.astype(jnp.bfloat16) if jnp.issubdtype(t.dtype, jnp.floating) else t)(jnp.asarray(a)))
    B, Hq, Hkv, Sq, Sk, D = 8, 32, 8, 112, 2048, 128
    return {
        "q": _w((lambda *s: _rng.normal(s) * 0.4)(B, Hq, Sq, D)),
        "k": _w((lambda *s: _rng.normal(s) * 0.4)(B, Hkv, Sk, D)),
        "v": _w((lambda *s: _rng.normal(s) * 0.05)(B, Hkv, Sk, D)),
    }

def reference(q, k, v):
    B, Hq, Sq, D = q.shape
    Hkv = k.shape[1]
    rep = Hq // Hkv
    k = jnp.repeat(k, rep, axis=1)
    v = jnp.repeat(v, rep, axis=1)
    scale = D ** -0.5
    scores = jnp.einsum("bhqd,bhkd->bhqk", q, k) * scale
    p = _softmax(scores, axis=-1)
    return jnp.einsum("bhqk,bhkd->bhqd", p, v)
```

```python
import functools, math
import jax, jax.numpy as jnp
from jax import lax
import jax.experimental.pallas as pl
import jax.experimental.pallas.tpu as pltpu
NT = (((1,), (1,)), ((), ()))
f32 = jnp.float32; bf16 = jnp.bfloat16

def ld(ref, u, r0, n):
    w = ref.bitcast(jnp.uint32)
    return pltpu.bitcast(w[u, r0//2:(r0+n)//2, :], bf16)

def _kernel(q_hbm, k_hbm, v_hbm, o_hbm, qb, kb, vb, ob, a_ref, sems, *, scale, mc, nb, lag, kg, G, plan):
    M = qb.shape[1]; Sk = kb.shape[1]
    nj = Sk // kg; ng = mc // 16; nch = M // mc
    def cp(kind, g, n):
        slot = g % nb
        if n > 1: slot = pl.multiple_of(slot, n)
        src = (q_hbm, k_hbm, v_hbm, ob)[kind]; dst = (qb, kb, vb, o_hbm)[kind]
        if kind == 3: return pltpu.make_async_copy(ob.at[pl.ds(slot, n)], o_hbm.at[pl.ds(g, n)], sems.at[3, slot])
        return pltpu.make_async_copy(src.at[pl.ds(g, n)], dst.at[pl.ds(slot, n)], sems.at[kind, slot])
    def fetch(g, n):
        for kind in range(3): cp(kind, g, n).start()
    BIG0, BS = plan[0], plan[1]

    def group(g0, size):
        big = size == BS
        if big:
            pl.when(g0 >= BIG0 + nb)(cp(3, jnp.maximum(g0 - nb, 0), BS).wait)
            @pl.when(jnp.logical_and(g0 >= nb, g0 < BIG0 + nb))
            def _():
                for u in range(BS): cp(3, jnp.maximum(g0 - nb, 0) + u, 1).wait()
            for kind in range(3): cp(kind, g0, BS).wait()
            pl.when(g0 + BS < G)(functools.partial(fetch, g0 + BS, BS))
        else:
            for u in range(size):
                for kind in range(3): cp(kind, g0 + u, 1).wait()
            for u in range(size):
                g = g0 + LA + u
                pl.when(g < BIG0)(functools.partial(fetch, g, 1))
            pl.when(g0 == plan[3])(functools.partial(fetch, BIG0, BS))
        za = g0 >> 16; zb = g0 >> 17
        chunks = [(u, i) for u in range(size) for i in range(nch)]
        n = len(chunks)
        slots = []
        for c in range(n + 1):
            if c < n: slots += [("qk", c, j) for j in range(nj)]
            if c >= 1: slots += [("pv", c - 1, j) for j in range(nj)]
        Q = {}; MP = {}; MX = {}; LP = {}; ACC = {}
        sl = [(g0 + u) % nb for u in range(size)]
        def retire(prev, g):
            kind, c, j, res = prev
            r = res[g*16:(g+1)*16]
            u, i = chunks[c]
            if kind == "qk":
                a_ref[za + c % 2, g*16:(g+1)*16, j*kg:(j+1)*kg] = r
                mx = r[:, 0:128]
                for t in range(1, kg // 128):
                    mx = jnp.maximum(mx, r[:, t*128:(t+1)*128])
                MP[c, g] = mx if j == 0 else jnp.maximum(MP[c, g], mx)
                if j == nj - 1:
                    MX[c, g] = jnp.max(MP.pop((c, g)), axis=1, keepdims=True)
            else:
                acc = r if j == 0 else ACC[c, g] + r
                if j == nj - 1:
                    l = jnp.sum(LP.pop((c, g)), axis=1, keepdims=True)
                    o = acc / l
                    ob[sl[u], i*mc + g*16:i*mc + (g+1)*16, :] = o.astype(ob.dtype)
                    a_ref[za + c % 2, g*16:(g+1)*16, Sk:Sk+128] = o
                else:
                    ACC[c, g] = acc
                    a_ref[za + c % 2, g*16:(g+1)*16, Sk:Sk+128] = acc
        pend = []
        for (kind, c, j) in slots:
            u, i = chunks[c]
            ps = []
            for g in range(ng):
                while len(pend) > max(lag - g - 1, 0):
                    retire(*pend.pop(0))
                if kind == "pv":
                    s = a_ref[zb + c % 2, g*16:(g+1)*16, j*kg:(j+1)*kg]
                    p = jnp.exp2(s - MX[c, g])
                    lp = p[:, 0:128]
                    for t in range(1, kg // 128):
                        lp = lp + p[:, t*128:(t+1)*128]
                    LP[c, g] = lp if j == 0 else LP[c, g] + lp
                    ps.append(p.astype(bf16))
            if kind == "qk":
                if j == 0:
                    q = ld(qb, sl[u], i*mc, mc)
                    Q[c] = (q.astype(f32) * scale).astype(bf16)
                res = lax.dot_general(Q[c], ld(kb, sl[u], j*kg, kg), NT, preferred_element_type=f32)
            else:
                res = jnp.dot(jnp.concatenate(ps, axis=0), ld(vb, sl[u], j*kg, kg), preferred_element_type=f32)
            for g in range(ng):
                pend.append(((kind, c, j, res), g))
        while pend:
            retire(*pend.pop(0))
        if big: cp(3, g0, BS).start()
        else:
            for u in range(size): cp(3, g0 + u, 1).start()

    LA = plan[2]
    for g in range(LA):
        fetch(g, 1)
    for (start, size, count) in plan[4]:
        def body(it, carry, start=start, size=size):
            group(start + it * size, size)
            return carry
        lax.fori_loop(0, count, body, 0)
    for g in range(G - nb, G, BS):
        cp(3, g, BS).wait()

PLAN_A = (8, 4, 4, 4, ((0, 1, 2), (2, 2, 3), (8, 4, 14)))
def make(mc=112, nb=16, lag=12, kg=512, plan=PLAN_A, flags=None, dbc=True):
    def f(q, k, v):
        B, Hq, Sq, D = q.shape
        Hkv, Sk = k.shape[1], k.shape[2]
        G = B * Hkv; M = (Hq // Hkv) * Sq
        q2 = q.reshape(G, M, D); k2 = k.reshape(G, Sk, D); v2 = v.reshape(G, Sk, D)
        scale = (D ** -0.5) * math.log2(math.e)
        out = pl.pallas_call(
            functools.partial(_kernel, scale=scale, mc=mc, nb=nb, lag=lag, kg=kg, G=G, plan=plan),
            grid=(1,),
            in_specs=[pl.BlockSpec(memory_space=pl.ANY)]*3,
            out_specs=pl.BlockSpec(memory_space=pl.ANY),
            out_shape=jax.ShapeDtypeStruct((G, M, D), q.dtype),
            scratch_shapes=[pltpu.VMEM((nb, M, D), bf16), pltpu.VMEM((nb, Sk, D), bf16), pltpu.VMEM((nb, Sk, D), bf16),
                            pltpu.VMEM((nb, M, D), bf16), pltpu.VMEM((2, mc, Sk + 128), f32),
                            pltpu.SemaphoreType.DMA((4, nb))],
            compiler_params=pltpu.CompilerParams(vmem_limit_bytes=100*1024*1024, flags=flags, disable_bounds_checks=dbc),
        )(q2, k2, v2)
        return out.reshape(B, Hq, Sq, D)
    return f


_impl = make()


@jax.jit
def pallas_standalone__gqa_softmax__near_ridge_kernel(q, k, v):
    return _impl(q, k, v)
```
